```python
import os as _os
_os.environ.setdefault("JAX_PLATFORMS", "cpu")
import jax
import jax.numpy as jnp

def _softmax(x, axis=-1):
    return jax.nn.softmax(x, axis=axis)
def _gelu(x):
    return jax.nn.gelu(x, approximate=True)
def _silu(x):
    return jax.nn.silu(x)
def _sigmoid(x):
    return jax.nn.sigmoid(x)
def _layernorm(x, axis=-1, eps=1e-5):
    m = jnp.mean(x, axis=axis, keepdims=True)
    v = jnp.var(x, axis=axis, keepdims=True)
    return (x - m) / jnp.sqrt(v + eps)
def _scatter_add(tgt, idx, src, axis=0):
    return tgt.at[idx].add(src)
def _segment_sum(src, seg, n):
    return jax.ops.segment_sum(src, seg, n)
class _Rng:
    def __init__(self, key):
        self._k = key
    def _next(self):
        self._k, sub = jax.random.split(self._k)
        return sub
    def normal(self, shape):
        return jax.random.normal(self._next(), shape, dtype=jnp.bfloat16)
    def randint(self, lo, hi, shape):
        return jax.random.randint(self._next(), shape, lo, hi, dtype=jnp.int32)
    def uniform(self, shape, lo=0.0, hi=1.0):
        return jax.random.uniform(self._next(), shape, jnp.bfloat16, lo, hi)
    def permutation(self, n):
        return jax.random.permutation(self._next(), n)


kernel_name = 'parallel_sum__linear_kernel_hedgehog__dense_activation_gelu__prompt'

def setup_inputs():
    _rng = _Rng(jax.random.key(int.from_bytes(__import__("os").urandom(4), "little")))
    _w = (lambda a: (lambda t: t.astype(jnp.bfloat16) if jnp.issubdtype(t.dtype, jnp.floating) else t)(jnp.asarray(a)))
    def _A_setup():
        B, S, D, H = 1, 2048, 448, 16
        Dh = D // H
        return {
            "x": _w((lambda *s: _rng.normal(s) * 0.05)(B, S, D)),
            "wqkv": _w((lambda *s: _rng.normal(s) * 0.2)(D, 3 * D)),
            "w_phi": _w((lambda *s: _rng.normal(s) * 0.2)(H, Dh, Dh) * (Dh ** -0.5)),
            "wo": _w((lambda *s: _rng.normal(s) * 0.05)(D, D)),
        }
    _A_in = _A_setup()

    def _B_setup():
        B, S, D, F = 1, 2048, 448, 1792
        return {
            "x": _w((lambda *s: _rng.normal(s) * 0.05)(B, S, D)),
            "w1": _w((lambda *s: _rng.normal(s) * 0.2)(D, F) * (D ** -0.5)),
            "b1": _w((lambda *s: _rng.normal(s) * 0.2)(F) * 0.01),
            "w2": _w((lambda *s: _rng.normal(s) * 0.2)(F, D) * (F ** -0.5)),
            "b2": _w((lambda *s: _rng.normal(s) * 0.05)(D) * 0.01),
        }
    _B_in = _B_setup()

    return {
        "A_x": _A_in["x"],
        "A_wqkv": _A_in["wqkv"],
        "A_w_phi": _A_in["w_phi"],
        "A_wo": _A_in["wo"],
        "B_x": _B_in["x"],
        "B_w1": _B_in["w1"],
        "B_b1": _B_in["b1"],
        "B_w2": _B_in["w2"],
        "B_b2": _B_in["b2"],
    }

def reference(A_x, A_wqkv, A_w_phi, A_wo, B_x, B_w1, B_b1, B_w2, B_b2):
    def _A_ref(x, wqkv, w_phi, wo):
        B, S, D = x.shape
        H = 16; Dh = D // H
        qkv = (lambda x, *d: x.transpose(*d))((x @ wqkv).reshape(B, S, 3, H, Dh), 2, 0, 3, 1, 4)
        q, k, v = qkv[0], qkv[1], qkv[2]
        pq = jnp.einsum("bhsd,hdf->bhsf", q, w_phi)
        pk = jnp.einsum("bhsd,hdf->bhsf", k, w_phi)
        phi_q = jnp.concatenate([_softmax(pq, axis=-1), _softmax(-pq, axis=-1)], axis=-1)
        phi_k = jnp.concatenate([_softmax(pk, axis=-1), _softmax(-pk, axis=-1)], axis=-1)
        kv = jnp.einsum("bhsf,bhsd->bhfd", phi_k, v)
        z  = jnp.einsum("bhsf->bhf", phi_k)
        num = jnp.einsum("bhqf,bhfd->bhqd", phi_q, kv)
        den = jnp.einsum("bhqf,bhf->bhq", phi_q, z)[..., None] + 1e-6
        o = num / den
        return (lambda x, *d: x.transpose(*d))(o, 0, 2, 1, 3).reshape(B, S, D) @ wo

    def _B_ref(x, w1, b1, w2, b2):
        h = jnp.einsum("bsd,df->bsf", x, w1) + b1
        h = _gelu(h)
        return jnp.einsum("bsf,fd->bsd", h, w2) + b2

    x = A_x
    xn = _layernorm(x, axis=-1)
    return x + _A_ref(xn, A_wqkv, A_w_phi, A_wo) + _B_ref(xn, B_w1, B_b1, B_w2, B_b2)
```

```python
import jax
import jax.numpy as jnp
import jax.experimental.pallas as pl
import jax.experimental.pallas.tpu as pltpu

T = 512
FC = 896
NN = (((1,), (0,)), ((), ()))
NT = (((1,), (1,)), ((), ()))
TN = (((0,), (0,)), ((), ()))


def _dot(a, b, dn=NN):
    return jax.lax.dot_general(a, b, dn, preferred_element_type=jnp.float32)


def _iota(shape, d):
    return jax.lax.broadcasted_iota(jnp.int32, shape, d)


def _phi(p):
    t = p.shape[1]
    p3 = p.reshape(14, 8, t)
    mx = jnp.max(p3, axis=0)
    mx = jnp.maximum(mx, pltpu.roll(mx, 4, 0))
    mn = jnp.min(p3, axis=0)
    mn = jnp.minimum(mn, pltpu.roll(mn, 4, 0))
    out = []
    for e in (jnp.exp(p3 - mx[None]), jnp.exp(mn[None] - p3)):
        s = jnp.sum(e, axis=0)
        s = s + pltpu.roll(s, 4, 0)
        out.append((e * (1.0 / s)[None]).reshape(112, t).astype(jnp.bfloat16))
    return jnp.concatenate(out, axis=0)


def _col(ref):
    return jnp.broadcast_to(ref[...].astype(jnp.float32), (128, ref.shape[1])).T


def _kernel(x_ref, wqkv_ref, wphi_ref, wo_h, w1_h, b1_ref, w2_h, b2_ref,
            o_ref, xn_s, acc_s, wq_s, wk_s, wv_s, wo_s, kvt_s, kvb_s, w1_s, b1_s, b2_s,
            wo_ref, w1_ref, w2_ref, sems):
    bf = jnp.bfloat16
    f32 = jnp.float32
    i = pl.program_id(0)
    n = pl.num_programs(0) // 2

    @pl.when(i == 0)
    def _():
        cps = [pltpu.make_async_copy(a, b, sems.at[k]) for k, (a, b) in
               enumerate(((wo_h, wo_ref), (w1_h, w1_ref), (w2_h, w2_ref)))]
        for cp in cps:
            cp.start()
        r = _iota((448, 28), 0)
        e = ((r % 112) // 4 == _iota((448, 28), 1)).astype(bf)
        bm = _dot(e, wphi_ref[...], NT)
        r = _iota((448, 448), 0)
        c = _iota((448, 448), 1)
        hr = (r // 112) * 4 + r % 4
        bm = jnp.where(hr == c // 28, bm, 0.0).astype(bf)
        wk_s[...] = _dot(bm, wqkv_ref[:, 448:896], NT).astype(bf)
        wq_s[...] = _dot(bm, wqkv_ref[:, 0:448], NT).astype(bf)
        perm = (hr * 28 + (r % 112) // 4 == c).astype(bf)
        wv_s[...] = _dot(perm, wqkv_ref[:, 896:1344], NT).astype(bf)
        cps[0].wait()
        wo_s[...] = _dot(perm, wo_ref[...]).T.astype(bf)
        b1_s[...] = _col(b1_ref)
        b2_s[...] = _col(b2_ref)
        kvt_s[...] = jnp.zeros_like(kvt_s)
        cps[1].wait()
        w1_s[...] = w1_ref[...].T
        cps[2].wait()

    @pl.when(i < n)
    def _():
        cols = pl.ds(pl.multiple_of(i * T, T), T)
        x = x_ref[...].astype(f32)
        m = jnp.mean(x, axis=0, keepdims=True)
        d = x - m
        var = jnp.mean(d * d, axis=0, keepdims=True)
        xn = (d * jax.lax.rsqrt(var + 1e-5)).astype(bf)
        xn_s[:, cols] = xn
        acc = x + jnp.tile(b2_s[...], (1, T // 128))
        for j in range(1792 // FC):
            sl = slice(j * FC, (j + 1) * FC)
            h = _dot(w1_s[sl, :], xn) + jnp.tile(b1_s[sl, :], (1, T // 128))
            h = jax.nn.gelu(h, approximate=True).astype(bf)
            acc = acc + _dot(w2_ref[:, sl], h)
        acc_s[:, cols] = acc
        v = _dot(wv_s[...], xn).astype(bf)
        pk = _dot(wk_s[...], xn)
        ones = jnp.ones((16, T), bf)
        for g in range(4):
            ph = _phi(pk[112 * g:112 * (g + 1)])
            vg = jnp.concatenate([v[112 * g:112 * (g + 1)], ones], axis=0)
            kvt_s[g] += _dot(vg, ph, NT)

    @pl.when(i == n)
    def _():
        keep = _iota((128, 224), 0) % 4 == _iota((128, 224), 1) % 4
        for g in range(4):
            kvb_s[g] = jnp.where(keep, kvt_s[g], 0.0).astype(bf)

    @pl.when(i >= n)
    def _():
        cols = pl.ds(pl.multiple_of((i - n) * T, T), T)
        xn = xn_s[:, cols]
        pq = _dot(wq_s[...], xn)
        os_ = []
        for g in range(4):
            ph = _phi(pq[112 * g:112 * (g + 1)])
            nd = _dot(kvb_s[g], ph)
            inv = 1.0 / (nd[112:120] + 1e-6)
            os_.append((nd[:112].reshape(14, 8, T) * inv[None]).reshape(112, T).astype(bf))
        ot = jnp.concatenate(os_, axis=0)
        o_ref[...] = (acc_s[:, cols] + _dot(wo_s[...], ot)).astype(o_ref.dtype)


@jax.jit
def pallas_parallel_sum__linear_kernel_hedgehog__dense_activation_gelu__prompt_kernel(
        A_x, A_wqkv, A_w_phi, A_wo, B_x, B_w1, B_b1, B_w2, B_b2):
    S, D = 2048, 448
    n = S // T
    bf = jnp.bfloat16
    args = (A_x.reshape(S, D).T, A_wqkv, A_w_phi.reshape(D, 28), A_wo, B_w1,
            B_b1.reshape(1, -1), B_w2.T, B_b2.reshape(1, -1))
    full = lambda a: pl.BlockSpec(a.shape, lambda i: (0, 0))
    out = pl.pallas_call(
        _kernel,
        grid=(2 * n,),
        in_specs=[pl.BlockSpec((D, T), lambda i: (0, jnp.minimum(i, n - 1)))]
        + [pl.BlockSpec(memory_space=pl.ANY) if k in (2, 3, 5) else full(a)
           for k, a in enumerate(args[1:])],
        out_specs=pl.BlockSpec((D, T), lambda i: (0, jnp.maximum(i - n, 0))),
        out_shape=jax.ShapeDtypeStruct((D, S), A_x.dtype),
        scratch_shapes=[
            pltpu.VMEM((D, S), bf), pltpu.VMEM((D, S), jnp.float32),
            pltpu.VMEM((D, D), bf), pltpu.VMEM((D, D), bf), pltpu.VMEM((D, D), bf),
            pltpu.VMEM((D, D), bf), pltpu.VMEM((4, 128, 224), jnp.float32),
            pltpu.VMEM((4, 128, 224), bf), pltpu.VMEM((1792, D), bf),
            pltpu.VMEM((1792, 128), jnp.float32), pltpu.VMEM((D, 128), jnp.float32),
            pltpu.VMEM((D, D), bf), pltpu.VMEM((D, 1792), bf), pltpu.VMEM((D, 1792), bf),
            pltpu.SemaphoreType.DMA((3,)),
        ],
        compiler_params=pltpu.CompilerParams(
            dimension_semantics=("arbitrary",), vmem_limit_bytes=64 * 1024 * 1024),
    )(*args)
    return out.T.reshape(1, S, D)
```
